```python
import os as _os
_os.environ.setdefault("JAX_PLATFORMS", "cpu")
import jax
import jax.numpy as jnp

def _softmax(x, axis=-1):
    return jax.nn.softmax(x, axis=axis)
def _gelu(x):
    return jax.nn.gelu(x, approximate=True)
def _silu(x):
    return jax.nn.silu(x)
def _sigmoid(x):
    return jax.nn.sigmoid(x)
def _layernorm(x, axis=-1, eps=1e-5):
    m = jnp.mean(x, axis=axis, keepdims=True)
    v = jnp.var(x, axis=axis, keepdims=True)
    return (x - m) / jnp.sqrt(v + eps)
def _scatter_add(tgt, idx, src, axis=0):
    return tgt.at[idx].add(src)
def _segment_sum(src, seg, n):
    return jax.ops.segment_sum(src, seg, n)
class _Rng:
    def __init__(self, key):
        self._k = key
    def _next(self):
        self._k, sub = jax.random.split(self._k)
        return sub
    def normal(self, shape):
        return jax.random.normal(self._next(), shape, dtype=jnp.bfloat16)
    def randint(self, lo, hi, shape):
        return jax.random.randint(self._next(), shape, lo, hi, dtype=jnp.int32)
    def uniform(self, shape, lo=0.0, hi=1.0):
        return jax.random.uniform(self._next(), shape, jnp.bfloat16, lo, hi)
    def permutation(self, n):
        return jax.random.permutation(self._next(), n)


kernel_name = 'parallel_sum__sliding_block_cached__dense_activation_mish__decode'

def setup_inputs():
    _rng = _Rng(jax.random.key(int.from_bytes(__import__("os").urandom(4), "little")))
    _w = (lambda a: (lambda t: t.astype(jnp.bfloat16) if jnp.issubdtype(t.dtype, jnp.floating) else t)(jnp.asarray(a)))
    def _A_setup():
        B, Sq, D = 2, 1, 512
        Hq, Hkv, Sk, Dh = 32, 8, 32768, 128
        assert Hq % Hkv == 0, (Hq, Hkv)
        return {
            "x": _w((lambda *s: _rng.normal(s) * 0.05)(B, Sq, D)),
            "k_cache": _w((lambda *s: _rng.normal(s) * 0.8)(B, Hkv, Sk, Dh)),
            "v_cache": _w((lambda *s: _rng.normal(s) * 0.8)(B, Hkv, Sk, Dh)),
            "wq": _w((lambda *s: _rng.normal(s) * 0.8)(D, Hq * Dh) * (D ** -0.5)),
            "wo": _w((lambda *s: _rng.normal(s) * 0.8)(Hq * Dh, D) * ((Hq * Dh) ** -0.5)),
        }
    _A_in = _A_setup()

    def _B_setup():
        B, S, D, F = 2, 1, 512, 1792
        return {
            "x": _w((lambda *s: _rng.normal(s) * 0.05)(B, S, D)),
            "w1": _w((lambda *s: _rng.normal(s) * 0.4)(D, F) * (D ** -0.5)),
            "b1": _w((lambda *s: _rng.normal(s) * 0.05)(F)),
            "w2": _w((lambda *s: _rng.normal(s) * 0.05)(F, D) * (F ** -0.5)),
        }
    _B_in = _B_setup()

    return {
        "A_x": _A_in["x"],
        "A_k_cache": _A_in["k_cache"],
        "A_v_cache": _A_in["v_cache"],
        "A_wq": _A_in["wq"],
        "A_wo": _A_in["wo"],
        "B_x": _B_in["x"],
        "B_w1": _B_in["w1"],
        "B_b1": _B_in["b1"],
        "B_w2": _B_in["w2"],
    }

def reference(A_x, A_k_cache, A_v_cache, A_wq, A_wo, B_x, B_w1, B_b1, B_w2):
    def _A_ref(x, k_cache, v_cache, wq, wo):
        B, Sq, D = x.shape
        Hq, Dh = 32, 128
        Hkv, Sk = k_cache.shape[1], k_cache.shape[2]
        W = min(4096, max(256, Sk // 4))
        rep = Hq // Hkv
        q = (lambda x, *d: x.transpose(*d))((x @ wq).reshape(B, Sq, Hq, Dh), 0, 2, 1, 3)
        k = jnp.repeat(k_cache[:, :, Sk - W:, :], rep, axis=1)
        v = jnp.repeat(v_cache[:, :, Sk - W:, :], rep, axis=1)
        scores = jnp.einsum("bhqd,bhkd->bhqk", q, k) * (Dh ** -0.5)
        p = _softmax(scores, axis=-1)
        o = jnp.einsum("bhqk,bhkd->bhqd", p, v)
        return (lambda x, *d: x.transpose(*d))(o, 0, 2, 1, 3).reshape(B, Sq, Hq * Dh) @ wo

    def _B_ref(x, w1, b1, w2):
        h = jnp.einsum("bsd,df->bsf", x, w1) + b1
        sp = jnp.log1p(jnp.exp(-jnp.abs(h))) + jnp.where(h > 0, h, jnp.zeros_like(h))
        act = h * jnp.tanh(sp)
        return jnp.einsum("bsf,fd->bsd", act, w2)

    x = A_x
    xn = _layernorm(x, axis=-1)
    return x + _A_ref(xn, A_k_cache, A_v_cache, A_wq, A_wo) + _B_ref(xn, B_w1, B_b1, B_w2)
```

```python
import jax
import jax.numpy as jnp
from jax import lax
import jax.experimental.pallas as pl
import jax.experimental.pallas.tpu as pltpu

_NT = (((1,), (1,)), ((), ()))
_NN = (((1,), (0,)), ((), ()))
_f32 = jnp.float32
_bf16 = jnp.bfloat16


@jax.jit
def pallas_parallel_sum__sliding_block_cached__dense_activation_mish__decode_kernel(
    A_x: jax.Array,
    A_k_cache: jax.Array,
    A_v_cache: jax.Array,
    A_wq: jax.Array,
    A_wo: jax.Array,
    B_x: jax.Array,
    B_w1: jax.Array,
    B_b1: jax.Array,
    B_w2: jax.Array,
):
    B, SQ, D = A_x.shape
    _, HKV, SK, DH = A_k_cache.shape
    HQ = A_wq.shape[1] // DH
    F = B_w1.shape[1]
    W = min(4096, max(256, SK // 4))
    REP = HQ // HKV
    GD = REP * DH
    R = B * REP
    assert SQ == 1 and B == 2 and R == 8

    def kernel(x_hbm, k_hbm, v_hbm, wq_hbm, wo_hbm, w1_hbm, b1_hbm, w2_hbm, o_ref,
               xbuf, b1buf, kbuf, vbuf, wqbuf, wobuf, w1buf, w2buf, q_scr, l_scr):
        def body(sems, ksems, vsems, osems):
            cx = pltpu.make_async_copy(x_hbm, xbuf, sems.at[0])
            cb1 = pltpu.make_async_copy(b1_hbm, b1buf, sems.at[1])
            cwq = pltpu.make_async_copy(wq_hbm, wqbuf, sems.at[2])
            cw1 = pltpu.make_async_copy(w1_hbm, w1buf, sems.at[3])
            cw2 = pltpu.make_async_copy(w2_hbm, w2buf, sems.at[4])

            def cwo(g):
                rows = pl.ds(pl.multiple_of(g * GD, GD), GD)
                return pltpu.make_async_copy(wo_hbm.at[rows, :], wobuf.at[rows, :], osems.at[g])

            def ck(g, b):
                return pltpu.make_async_copy(k_hbm.at[b, g, pl.ds(SK - W, W), :],
                                             kbuf.at[g * B + b], ksems.at[g * B + b])

            def cv(g, b):
                return pltpu.make_async_copy(v_hbm.at[b, g, pl.ds(SK - W, W), :],
                                             vbuf.at[g * B + b], vsems.at[g * B + b])

            cx.start()
            cwq.start()
            cb1.start()

            def issue(i, c):
                g, b = i // B, i % B
                ck(g, b).start()
                cv(g, b).start()
                return c
            lax.fori_loop(0, B * HKV, issue, 0)

            cx.wait()
            cw1.start()
            cw2.start()
            x = xbuf[...].astype(_f32)
            row = lax.broadcasted_iota(jnp.int32, (R, D), 0)
            x8 = jnp.where(row < REP, jnp.broadcast_to(x[0:1, :], (R, D)),
                           jnp.broadcast_to(x[1:2, :], (R, D)))
            mu = jnp.mean(x8, axis=-1, keepdims=True)
            xc = x8 - mu
            var = jnp.mean(xc * xc, axis=-1, keepdims=True)
            xn8 = (xc * lax.rsqrt(var + 1e-5)).astype(_bf16)

            cwq.wait()
            r = lax.dot_general(xn8, wqbuf[...], _NN, preferred_element_type=_f32)
            r = r * (DH ** -0.5)
            rj = lax.broadcasted_iota(jnp.int32, (R, DH), 0) % REP
            for g in range(HKV):
                qg = jnp.zeros((R, DH), _f32)
                for j in range(REP):
                    c = (g * REP + j) * DH
                    qg = jnp.where(rj == j, r[:, c:c + DH], qg)
                q_scr[g] = qg

            rowb = lax.broadcasted_iota(jnp.int32, (R, DH), 0) // REP

            def gloop(g, carry):
                cwo(g).start()
                qg = q_scr[g].astype(_bf16)
                outs = []
                for b in range(B):
                    i = g * B + b
                    ck(g, b).wait()
                    s = lax.dot_general(qg, kbuf[i], _NT, preferred_element_type=_f32)
                    m = jnp.max(s, axis=-1, keepdims=True)
                    p = jnp.exp(s - m)
                    l = jnp.sum(p, axis=-1, keepdims=True)
                    pb = p.astype(_bf16)
                    cv(g, b).wait()
                    o = lax.dot_general(pb, vbuf[i], _NN, preferred_element_type=_f32)
                    outs.append(o / l)
                og = jnp.where(rowb == 0, outs[0], outs[1])
                l_scr[g] = jnp.concatenate(
                    [jnp.where(rj == j, og, 0.0) for j in range(REP)], axis=-1)
                return carry
            lax.fori_loop(0, HKV, gloop, 0)

            cw1.wait()
            cb1.wait()
            b1 = b1buf[...].astype(_f32).reshape(1, F)
            h = lax.dot_general(xn8, w1buf[...], _NN, preferred_element_type=_f32) + b1
            sp = jnp.log1p(jnp.exp(-jnp.abs(h))) + jnp.maximum(h, 0.0)
            act = (h * jnp.tanh(sp)).astype(_bf16)
            cw2.wait()
            y = lax.dot_general(act, w2buf[...], _NN, preferred_element_type=_f32) + x8
            y = jnp.where(row % REP == 0, y, 0.0)
            for g in range(HKV):
                cwo(g).wait()
                y = y + lax.dot_general(l_scr[g].astype(_bf16), wobuf[g * GD:(g + 1) * GD, :],
                                        _NN, preferred_element_type=_f32)
            o0 = jnp.sum(y[0:REP, :], axis=0, keepdims=True)
            o1 = jnp.sum(y[REP:R, :], axis=0, keepdims=True)
            o_ref[...] = jnp.concatenate([o0, o1], axis=0).astype(o_ref.dtype)

        pl.run_scoped(body,
                      pltpu.SemaphoreType.DMA((5,)),
                      pltpu.SemaphoreType.DMA((B * HKV,)),
                      pltpu.SemaphoreType.DMA((B * HKV,)),
                      pltpu.SemaphoreType.DMA((HKV,)))

    anyspec = pl.BlockSpec(memory_space=pl.ANY)
    out = pl.pallas_call(
        kernel,
        out_shape=jax.ShapeDtypeStruct((B, D), A_x.dtype),
        in_specs=[anyspec] * 8,
        out_specs=pl.BlockSpec(memory_space=pltpu.VMEM),
        scratch_shapes=[
            pltpu.VMEM((B, D), _bf16),
            pltpu.VMEM((F,), _bf16),
            pltpu.VMEM((B * HKV, W, DH), _bf16),
            pltpu.VMEM((B * HKV, W, DH), _bf16),
            pltpu.VMEM((D, HQ * DH), _bf16),
            pltpu.VMEM((HQ * DH, D), _bf16),
            pltpu.VMEM((D, F), _bf16),
            pltpu.VMEM((F, D), _bf16),
            pltpu.VMEM((HKV, R, DH), _f32),
            pltpu.VMEM((HKV, R, GD), _f32),
        ],
        compiler_params=pltpu.CompilerParams(vmem_limit_bytes=100 * 1024 * 1024),
    )(A_x.reshape(B, D), A_k_cache, A_v_cache, A_wq, A_wo, B_w1, B_b1, B_w2)
    return out.reshape(B, SQ, D)
```

```python
import jax
import jax.numpy as jnp
from jax import lax
import jax.experimental.pallas as pl
import jax.experimental.pallas.tpu as pltpu

_NT = (((1,), (1,)), ((), ()))
_NN = (((1,), (0,)), ((), ()))
_f32 = jnp.float32
_bf16 = jnp.bfloat16

_TAIL = (256, 128, 80, 32, 16)


@jax.jit
def pallas_parallel_sum__sliding_block_cached__dense_activation_mish__decode_kernel(
    A_x: jax.Array,
    A_k_cache: jax.Array,
    A_v_cache: jax.Array,
    A_wq: jax.Array,
    A_wo: jax.Array,
    B_x: jax.Array,
    B_w1: jax.Array,
    B_b1: jax.Array,
    B_w2: jax.Array,
):
    B, SQ, D = A_x.shape
    _, HKV, SK, DH = A_k_cache.shape
    HQ = A_wq.shape[1] // DH
    F = B_w1.shape[1]
    W = min(4096, max(256, SK // 4))
    REP = HQ // HKV
    GD = REP * DH
    R = B * REP
    NT = len(_TAIL)
    assert SQ == 1 and B == 2 and R == 8 and sum(_TAIL) == GD and DH == 128
    assert NT <= HKV + 2
    tail_off = [sum(_TAIL[:t]) for t in range(NT)]
    scale = DH ** -0.5

    def kernel(x_hbm, k_hbm, v_hbm, wq_hbm, wo_hbm, w1_hbm, b1_hbm, w2_hbm, o_ref,
               xbuf, b1buf, kbuf, vbuf, wqbuf, wobuf, w1buf, w2buf,
               q_scr, og_scr, coef_scr, *tailbufs):

        def body(sems, ksems, vsems, osems, tsems):
            cx = pltpu.make_async_copy(x_hbm, xbuf, sems.at[0])
            cb1 = pltpu.make_async_copy(b1_hbm, b1buf, sems.at[1])
            cwq = pltpu.make_async_copy(wq_hbm, wqbuf, sems.at[2])
            cw1 = pltpu.make_async_copy(w1_hbm, w1buf, sems.at[3])
            cw2 = pltpu.make_async_copy(w2_hbm, w2buf, sems.at[4])

            def ck(g, b):
                return pltpu.make_async_copy(k_hbm.at[b, g, pl.ds(SK - W, W), :],
                                             kbuf.at[g * B + b], ksems.at[g * B + b])

            def cv(g, b):
                return pltpu.make_async_copy(v_hbm.at[b, g, pl.ds(SK - W, W), :],
                                             vbuf.at[g * B + b], vsems.at[g * B + b])

            def cwo(g):
                rows = pl.ds(pl.multiple_of(g * GD, GD), GD)
                return pltpu.make_async_copy(wo_hbm.at[rows, :], wobuf.at[g], osems.at[g])

            def ct(t):
                rows = pl.ds((HKV - 1) * GD + tail_off[t], _TAIL[t])
                return pltpu.make_async_copy(wo_hbm.at[rows, :], tailbufs[t], tsems.at[t])

            cx.start()
            cwq.start()
            cb1.start()

            def issue(g, c):
                for b in range(B):
                    ck(g, b).start()
                    cv(g, b).start()
                return c
            lax.fori_loop(0, HKV, issue, 0)

            cx.wait()
            cw1.start()
            cw2.start()
            x = xbuf[...].astype(_f32)
            row = lax.broadcasted_iota(jnp.int32, (R, D), 0)
            x8 = jnp.where(row < REP, jnp.broadcast_to(x[0:1, :], (R, D)),
                           jnp.broadcast_to(x[1:2, :], (R, D)))
            mu = jnp.mean(x8, axis=-1, keepdims=True)
            xc = x8 - mu
            var = jnp.mean(xc * xc, axis=-1, keepdims=True)
            xn8 = (xc * lax.rsqrt(var + 1e-5)).astype(_bf16)

            cwq.wait()
            qall = lax.dot_general(xn8, wqbuf[...], _NN, preferred_element_type=_f32)
            rowh = lax.broadcasted_iota(jnp.int32, (R, DH), 0)
            rj = rowh % REP
            for g in range(HKV):
                qg = qall[:, g * GD:g * GD + DH]
                for j in range(1, REP):
                    c = g * GD + j * DH
                    qg = jnp.where(rj == j, qall[:, c:c + DH], qg)
                q_scr[g] = qg

            def gloop(g, carry):
                @pl.when(g < HKV - 1)
                def _():
                    cwo(g).start()
                qg = q_scr[g].astype(_bf16)
                outs = []
                for b in range(B):
                    i = g * B + b
                    ck(g, b).wait()
                    s = lax.dot_general(qg, kbuf[i], _NT, preferred_element_type=_f32) * scale
                    m = jnp.max(s, axis=-1, keepdims=True)
                    p = jnp.exp(s - m)
                    l = jnp.sum(p, axis=-1, keepdims=True)
                    pb = p.astype(_bf16)
                    cv(g, b).wait()
                    o = lax.dot_general(pb, vbuf[i], _NN, preferred_element_type=_f32)
                    outs.append(o / l)
                og_scr[g] = jnp.where(rowh < REP, outs[0], outs[1])
                return carry
            lax.fori_loop(0, HKV, gloop, 0)

            nxt = [0]

            def issue_tail():
                if nxt[0] < NT:
                    ct(nxt[0]).start()
                    nxt[0] += 1

            issue_tail()
            ogl = og_scr[HKV - 1].astype(_bf16).astype(_f32)
            for b in range(B):
                for j in range(REP):
                    rr = b * REP + j
                    coef_scr[b, j * DH:(j + 1) * DH, :] = jnp.transpose(
                        jnp.broadcast_to(ogl[rr:rr + 1, :], (DH, DH)))

            cw1.wait()
            cb1.wait()
            issue_tail()
            b1 = b1buf[...].astype(_f32).reshape(1, F)
            h = lax.dot_general(xn8, w1buf[...], _NN, preferred_element_type=_f32) + b1
            sp = jnp.log1p(jnp.exp(-jnp.abs(h))) + jnp.maximum(h, 0.0)
            act = (h * jnp.tanh(sp)).astype(_bf16)
            cw2.wait()
            issue_tail()
            y = lax.dot_general(act, w2buf[...], _NN, preferred_element_type=_f32) + x8
            y = jnp.where(row % REP == 0, y, 0.0)

            for g in range(HKV - 1):
                og = og_scr[g]
                lhs = jnp.concatenate(
                    [jnp.where(rj == j, og, 0.0) for j in range(REP)], axis=-1).astype(_bf16)
                cwo(g).wait()
                issue_tail()
                y = y + lax.dot_general(lhs, wobuf[g], _NN, preferred_element_type=_f32)
            assert nxt[0] == NT

            z = [jnp.where(row < REP, y, 0.0), jnp.where(row < REP, 0.0, y)]
            for t in range(NT):
                ct(t).wait()
                for r0 in range(0, _TAIL[t], 8):
                    wrow = tailbufs[t][r0:r0 + 8, :].astype(_f32)
                    c0 = tail_off[t] + r0
                    for b in range(B):
                        cb = coef_scr[b, c0:c0 + 8, :]
                        z[b] = z[b] + wrow * jnp.concatenate([cb] * (D // DH), axis=-1)

            t0 = jnp.where(row < REP, z[0] + pltpu.roll(z[0], 4, 0),
                           z[1] + pltpu.roll(z[1], 4, 0))
            t1 = t0 + pltpu.roll(t0, 6, 0)
            t2 = t1 + pltpu.roll(t1, 7, 0)
            res = jnp.where(row == 0, t2, pltpu.roll(t2, 5, 0))
            o_ref[...] = res[0:B, :].astype(o_ref.dtype)

        pl.run_scoped(body,
                      pltpu.SemaphoreType.DMA((5,)),
                      pltpu.SemaphoreType.DMA((B * HKV,)),
                      pltpu.SemaphoreType.DMA((B * HKV,)),
                      pltpu.SemaphoreType.DMA((HKV - 1,)),
                      pltpu.SemaphoreType.DMA((NT,)))

    anyspec = pl.BlockSpec(memory_space=pl.ANY)
    out = pl.pallas_call(
        kernel,
        out_shape=jax.ShapeDtypeStruct((B, D), A_x.dtype),
        in_specs=[anyspec] * 8,
        out_specs=pl.BlockSpec(memory_space=pltpu.VMEM),
        scratch_shapes=[
            pltpu.VMEM((B, D), A_x.dtype),
            pltpu.VMEM((F,), B_b1.dtype),
            pltpu.VMEM((B * HKV, W, DH), A_k_cache.dtype),
            pltpu.VMEM((B * HKV, W, DH), A_v_cache.dtype),
            pltpu.VMEM((D, HQ * DH), A_wq.dtype),
            pltpu.VMEM((HKV - 1, GD, D), A_wo.dtype),
            pltpu.VMEM((D, F), B_w1.dtype),
            pltpu.VMEM((F, D), B_w2.dtype),
            pltpu.VMEM((HKV, R, DH), _f32),
            pltpu.VMEM((HKV, R, DH), _f32),
            pltpu.VMEM((B, GD, DH), _f32),
        ] + [pltpu.VMEM((n, D), A_wo.dtype) for n in _TAIL],
        compiler_params=pltpu.CompilerParams(vmem_limit_bytes=64 * 1024 * 1024),
    )(A_x.reshape(B, D), A_k_cache, A_v_cache, A_wq, A_wo, B_w1, B_b1, B_w2)
    return out.reshape(B, SQ, D)
```
